```python
import os as _os
_os.environ.setdefault("JAX_PLATFORMS", "cpu")
import jax
import jax.numpy as jnp

def _softmax(x, axis=-1):
    return jax.nn.softmax(x, axis=axis)
def _gelu(x):
    return jax.nn.gelu(x, approximate=True)
def _silu(x):
    return jax.nn.silu(x)
def _sigmoid(x):
    return jax.nn.sigmoid(x)
def _layernorm(x, axis=-1, eps=1e-5):
    m = jnp.mean(x, axis=axis, keepdims=True)
    v = jnp.var(x, axis=axis, keepdims=True)
    return (x - m) / jnp.sqrt(v + eps)
def _scatter_add(tgt, idx, src, axis=0):
    return tgt.at[idx].add(src)
def _segment_sum(src, seg, n):
    return jax.ops.segment_sum(src, seg, n)
class _Rng:
    def __init__(self, key):
        self._k = key
    def _next(self):
        self._k, sub = jax.random.split(self._k)
        return sub
    def normal(self, shape):
        return jax.random.normal(self._next(), shape, dtype=jnp.bfloat16)
    def randint(self, lo, hi, shape):
        return jax.random.randint(self._next(), shape, lo, hi, dtype=jnp.int32)
    def uniform(self, shape, lo=0.0, hi=1.0):
        return jax.random.uniform(self._next(), shape, jnp.bfloat16, lo, hi)
    def permutation(self, n):
        return jax.random.permutation(self._next(), n)


kernel_name = 'concat_heads__mha_block_cached__gqa_block_cached__near_ridge'

def setup_inputs():
    _rng = _Rng(jax.random.key(int.from_bytes(__import__("os").urandom(4), "little")))
    _w = (lambda a: (lambda t: t.astype(jnp.bfloat16) if jnp.issubdtype(t.dtype, jnp.floating) else t)(jnp.asarray(a)))
    def _A_setup():
        B, Sq, D = 8, 128, 512
        H, Sk, Dh = 32, 1024, 128
        return {
            "x": _w((lambda *s: _rng.normal(s) * 0.8)(B, Sq, D)),
            "k_cache": _w((lambda *s: _rng.normal(s) * 0.8)(B, H, Sk, Dh)),
            "v_cache": _w((lambda *s: _rng.normal(s) * 0.05)(B, H, Sk, Dh)),
            "wq": _w((lambda *s: _rng.normal(s) * 0.8)(D, H * Dh) * (D ** -0.5)),
            "wo": _w((lambda *s: _rng.normal(s) * 0.05)(H * Dh, D) * ((H * Dh) ** -0.5)),
        }
    _A_in = _A_setup()

    def _B_setup():
        B, Sq, D = 8, 128, 512
        Hq, Hkv, Sk, Dh = 32, 32, 1024, 128
        assert Hq % Hkv == 0, (Hq, Hkv)
        return {
            "x": _w((lambda *s: _rng.normal(s) * 0.8)(B, Sq, D)),
            "k_cache": _w((lambda *s: _rng.normal(s) * 0.8)(B, Hkv, Sk, Dh)),
            "v_cache": _w((lambda *s: _rng.normal(s) * 0.05)(B, Hkv, Sk, Dh)),
            "wq": _w((lambda *s: _rng.normal(s) * 0.8)(D, Hq * Dh) * (D ** -0.5)),
            "wo": _w((lambda *s: _rng.normal(s) * 0.05)(Hq * Dh, D) * ((Hq * Dh) ** -0.5)),
        }
    _B_in = _B_setup()

    return {
        "A_x": _A_in["x"],
        "A_k_cache": _A_in["k_cache"],
        "A_v_cache": _A_in["v_cache"],
        "A_wq": _A_in["wq"],
        "A_wo": _A_in["wo"],
        "B_x": _B_in["x"],
        "B_k_cache": _B_in["k_cache"],
        "B_v_cache": _B_in["v_cache"],
        "B_wq": _B_in["wq"],
        "B_wo": _B_in["wo"],
    }

def reference(A_x, A_k_cache, A_v_cache, A_wq, A_wo, B_x, B_k_cache, B_v_cache, B_wq, B_wo):
    def _A_ref(x, k_cache, v_cache, wq, wo):
        B, Sq, D = x.shape
        H, Dh = 32, 128
        q = (lambda x, *d: x.transpose(*d))((x @ wq).reshape(B, Sq, H, Dh), 0, 2, 1, 3)
        scores = jnp.einsum("bhqd,bhkd->bhqk", q, k_cache) * (Dh ** -0.5)
        p = _softmax(scores, axis=-1)
        o = jnp.einsum("bhqk,bhkd->bhqd", p, v_cache)
        return (lambda x, *d: x.transpose(*d))(o, 0, 2, 1, 3).reshape(B, Sq, H * Dh) @ wo

    def _B_ref(x, k_cache, v_cache, wq, wo):
        B, Sq, D = x.shape
        Hq, Dh = 32, 128
        Hkv = k_cache.shape[1]
        rep = Hq // Hkv
        q = (lambda x, *d: x.transpose(*d))((x @ wq).reshape(B, Sq, Hq, Dh), 0, 2, 1, 3)
        k = jnp.repeat(k_cache, rep, axis=1)
        v = jnp.repeat(v_cache, rep, axis=1)
        scores = jnp.einsum("bhqd,bhkd->bhqk", q, k) * (Dh ** -0.5)
        p = _softmax(scores, axis=-1)
        o = jnp.einsum("bhqk,bhkd->bhqd", p, v)
        return (lambda x, *d: x.transpose(*d))(o, 0, 2, 1, 3).reshape(B, Sq, Hq * Dh) @ wo

    a = _A_ref(A_x, A_k_cache, A_v_cache, A_wq, A_wo)
    b = _B_ref(B_x, B_k_cache, B_v_cache, B_wq, B_wo)
    return jnp.concatenate([a, b], axis=-1)
```

```python
import functools, math

import jax
import jax.numpy as jnp
import jax.experimental.pallas as pl
import jax.experimental.pallas.tpu as pltpu

_NT = (((1,), (1,)), ((), ()))
HB = 2
NSLOT = 3
LANE = 128
CH = 128
ORDER = 1
DMA_ONLY = False


def _kernel(xa, ka, va, wqa, woa, xb, kb, vb, wqb, wob,
            out,
            x_v, wq_v, wo_v, kv_v, acc, o_v,
            sem_x, sem_wq, sem_wo, sem_kv, sem_o,
            *, B, Sq, D, H, Sk, Dh, hb, nslot):
    ng = H // hb
    nsteps = ng * B
    nkt = D // LANE
    c = (Dh ** -0.5) * math.log2(math.e)
    xs, wqs, wos = (xa, xb), (wqa, wqb), (woa, wob)
    kvs = (ka, kb, va, vb)
    nch = Sk // CH

    def start_x():
        for kt in range(nkt):
            for b in range(B):
                for i in range(2):
                    pltpu.make_async_copy(xs[i].at[b, :, pl.ds(kt * LANE, LANE)], x_v.at[i, kt, b], sem_x).start(priority=i)

    def wait_x():
        pltpu.make_async_copy(x_v, x_v, sem_x).wait()

    def start_wq(g):
        for h in range(hb):
            for r in range(D // CH):
                for i in range(2):
                    pltpu.make_async_copy(
                        wqs[i].at[pl.ds(r * CH, CH), pl.ds(pl.multiple_of((g * hb + h) * Dh, Dh), Dh)],
                        wq_v.at[i, g * hb + h, pl.ds(r * CH, CH)], sem_wq.at[g]).start(priority=i)

    def wait_wq(g):
        v = wq_v.at[:, pl.ds(g * hb, hb)]
        pltpu.make_async_copy(v, v, sem_wq.at[g]).wait()

    def start_wo(g):
        for j in range(nkt):
            for r in range(hb * Dh // CH):
                r0 = pl.multiple_of(g * hb * Dh + r * CH, CH)
                for i in range(2):
                    pltpu.make_async_copy(
                        wos[i].at[pl.ds(r0, CH), pl.ds(j * LANE, LANE)],
                        wo_v.at[i, j, pl.ds(r0, CH)], sem_wo.at[g]).start(priority=i)

    def wait_wo(g):
        v = wo_v.at[:, :, pl.ds(pl.multiple_of(g * hb * Dh, hb * Dh), hb * Dh)]
        pltpu.make_async_copy(v, v, sem_wo.at[g]).wait()

    def start_kv(t):
        g, b, slot = t // B, t % B, t % nslot
        def one(a, h, ci, pr):
            pltpu.make_async_copy(kvs[a].at[b, g * hb + h, pl.ds(ci * CH, CH)],
                                  kv_v.at[slot, a, h, pl.ds(ci * CH, CH)], sem_kv.at[slot, a]).start(priority=pr)
        if ORDER == 1:
            for h in range(hb):
                for ci in range(nch):
                    for a in (0, 2, 1, 3):
                        one(a, h, ci, a // 2)
        elif ORDER == 2:
            for i in range(2):
                for h in range(hb):
                    for ci in range(nch):
                        one(i, h, ci, 0)
                        one(2 + i, h, ci, 1)
        elif ORDER == 3:
            for h in range(hb):
                for kv in range(2):
                    for ci in range(nch):
                        one(2 * kv, h, ci, 0)
                        one(2 * kv + 1, h, ci, 1)

    def wait_kv(t):
        slot = t % nslot
        for a in range(4):
            pltpu.make_async_copy(kv_v.at[slot, a], kv_v.at[slot, a], sem_kv.at[slot, a]).wait()

    def out_copy(b):
        return pltpu.make_async_copy(o_v.at[b], out.at[b], sem_o.at[b])

    def issue(t):
        first = (t % B) == 0
        g = t // B
        if isinstance(t, int):
            if first: start_wq(g)
            start_kv(t)
            if first: start_wo(g)
        else:
            @pl.when(first)
            def _():
                start_wq(g)
            start_kv(t)
            @pl.when(first)
            def _():
                start_wo(g)

    start_x()
    for t in range(nslot - 1):
        issue(t)
    acc[...] = jnp.zeros(acc.shape, acc.dtype)
    wait_x()

    def step(s, carry):
        g, b, slot = s // B, s % B, s % nslot

        @pl.when(s + nslot - 1 < nsteps)
        def _():
            issue(s + nslot - 1)

        @pl.when(b == 0)
        def _():
            wait_wq(g)
            wait_wo(g)

        wait_kv(s)

        if DMA_ONLY:
            acc[b, :, 0:128] += (kv_v[slot, 0, 0, 0:128, :] + kv_v[slot, 1, 0, 0:128, :] + kv_v[slot, 2, 0, 0:128, :] + kv_v[slot, 3, 0, 0:128, :]).astype(jnp.float32)
        else:
            items = [(i, h) for i in range(2) for h in range(hb)]
            xcat = [jnp.concatenate([x_v[i, kt, b] for kt in range(nkt)], axis=1) for i in range(2)]

            def qk(j):
                i, h = items[j]
                q = jnp.dot(xcat[i], wq_v[i, g * hb + h], preferred_element_type=jnp.float32)
                q = (q * c).astype(jnp.bfloat16)
                return jax.lax.dot_general(q, kv_v[slot, i, h], _NT, preferred_element_type=jnp.float32)

            outs = [[], []]
            s_next = qk(0)
            for j, (i, h) in enumerate(items):
                sc = s_next
                if j + 1 < len(items):
                    s_next = qk(j + 1)
                m = jnp.max(sc, axis=-1, keepdims=True)
                p = jnp.exp2(sc - m)
                l = jnp.sum(p, axis=-1, keepdims=True)
                o = jnp.dot(p.astype(jnp.bfloat16), kv_v[slot, 2 + i, h], preferred_element_type=jnp.float32)
                o = o * pl.reciprocal(l, approx=False)
                outs[i].append(o.astype(jnp.bfloat16))
                if h == hb - 1:
                    oc = jnp.concatenate(outs[i], axis=-1)
                    r0 = pl.multiple_of(g * hb * Dh, hb * Dh)
                    for jj in range(nkt):
                        col = i * D + jj * LANE
                        acc[b, :, col:col + LANE] += jnp.dot(
                            oc, wo_v[i, jj, pl.ds(r0, hb * Dh), :], preferred_element_type=jnp.float32)

        @pl.when(g == ng - 1)
        def _():
            o_v[b] = acc[b].astype(o_v.dtype)
            out_copy(b).start()
        return carry

    jax.lax.fori_loop(0, nsteps, step, 0)
    for b in range(B):
        out_copy(b).wait()


@jax.jit
def pallas_concat_heads__mha_block_cached__gqa_block_cached__near_ridge_kernel(
    A_x, A_k_cache, A_v_cache, A_wq, A_wo,
    B_x, B_k_cache, B_v_cache, B_wq, B_wo,
):
    B, Sq, D = A_x.shape
    _, H, Sk, Dh = A_k_cache.shape
    hb, nslot = HB, NSLOT
    ng = H // hb
    nkt = D // LANE
    bf = jnp.bfloat16
    return pl.pallas_call(
        functools.partial(_kernel, B=B, Sq=Sq, D=D, H=H, Sk=Sk, Dh=Dh, hb=hb, nslot=nslot),
        in_specs=[pl.BlockSpec(memory_space=pl.ANY)] * 10,
        out_specs=pl.BlockSpec(memory_space=pl.ANY),
        out_shape=jax.ShapeDtypeStruct((B, Sq, 2 * D), bf),
        scratch_shapes=[
            pltpu.VMEM((2, nkt, B, Sq, LANE), bf),
            pltpu.VMEM((2, H, D, Dh), bf),
            pltpu.VMEM((2, nkt, H * Dh, LANE), bf),
            pltpu.VMEM((nslot, 4, hb, Sk, Dh), bf),
            pltpu.VMEM((B, Sq, 2 * D), jnp.float32),
            pltpu.VMEM((B, Sq, 2 * D), bf),
            pltpu.SemaphoreType.DMA(()),
            pltpu.SemaphoreType.DMA((ng,)),
            pltpu.SemaphoreType.DMA((ng,)),
            pltpu.SemaphoreType.DMA((nslot, 4)),
            pltpu.SemaphoreType.DMA((B,)),
        ],
        compiler_params=pltpu.CompilerParams(vmem_limit_bytes=100 * 1024 * 1024, disable_bounds_checks=True),
    )(A_x, A_k_cache, A_v_cache, A_wq, A_wo,
      B_x, B_k_cache, B_v_cache, B_wq, B_wo)
```

```python
import functools
import math

import jax
import jax.numpy as jnp
import jax.experimental.pallas as pl
import jax.experimental.pallas.tpu as pltpu

_NT = (((1,), (1,)), ((), ()))
LANE = 128
NB = 4
CH = 32
NPART = 4
SHIFT = 8
NSLOT = 4
FLUSH_J = 1


def _kernel(xa, ka, va, wqa, woa, xb, kb, vb, wqb, wob,
            out,
            x_v, wq_v, wo_v, kv_v, acc, o_v,
            sems, sem_o,
            *, B, Sq, D, H, Sk, Dh, reps):
    nb, nslot = NB, NSLOT
    nbg = B // nb
    npair = H * nbg
    nkt = D // LANE
    cpp = Sk // CH // NPART
    c = (Dh ** -0.5) * math.log2(math.e)
    xs, wqs, wos = (xa, xb), (wqa, wqb), (woa, wob)
    ks, vs = (ka, kb), (va, vb)

    def sem_kv(slot, a):
        return sems.at[2 * slot + a]

    def sem_w(i, par):
        return sems.at[2 * nslot + 2 * i + par]

    def sem_x(i, bg):
        return sems.at[2 * nslot + 4 + i * nbg + bg]

    def wait_all(view, sem):
        pltpu.make_async_copy(view, view, sem).wait()

    def row0(h):
        return h * Dh if isinstance(h, int) else pl.multiple_of(h * Dh, Dh)

    def start_x(i, bg):
        for kt in range(nkt):
            for j in range(nb):
                b = bg * nb + j
                pltpu.make_async_copy(
                    xs[i].at[b, :, pl.ds(kt * LANE, LANE)], x_v.at[i, kt, b],
                    sem_x(i, bg)).start(priority=j % 2)

    def wait_x(i, bg):
        wait_all(x_v.at[i, :, pl.ds(bg * nb, nb)], sem_x(i, bg))

    def start_w(i, h):
        r0 = row0(h)
        for r in range(nkt):
            pltpu.make_async_copy(
                wqs[i].at[pl.ds(r * LANE, LANE), pl.ds(r0, Dh)],
                wq_v.at[i, h, pl.ds(r * LANE, LANE)],
                sem_w(i, h % 2)).start(priority=0)
            pltpu.make_async_copy(
                wos[i].at[pl.ds(r0, Dh), pl.ds(r * LANE, LANE)],
                wo_v.at[i, r, pl.ds(r0, Dh)],
                sem_w(i, h % 2)).start(priority=1)

    def wait_w(i, h):
        wait_all(wq_v.at[i, h], sem_w(i, h % 2))
        wait_all(wo_v.at[i, :, pl.ds(row0(h), Dh)], sem_w(i, h % 2))

    def start_kv(i, p, part):
        h, bg, slot = p // nbg, p % nbg, (2 * p + i) % nslot
        hkv = h if reps[i] == 1 else h // reps[i]
        for ci in range(part * cpp, (part + 1) * cpp):
            for a, arr in enumerate((ks[i], vs[i])):
                pltpu.make_async_copy(
                    arr.at[pl.ds(bg * nb, nb), hkv, pl.ds(ci * CH, CH)],
                    kv_v.at[slot, a, :, pl.ds(ci * CH, CH)],
                    sem_kv(slot, a)).start(priority=a)

    def wait_kv(i, p):
        slot = (2 * p + i) % nslot
        for a in range(2):
            wait_all(kv_v.at[slot, a], sem_kv(slot, a))

    def out_copy(i, b):
        return pltpu.make_async_copy(
            o_v.at[b, :, pl.ds(i * D, D)], out.at[b, :, pl.ds(i * D, D)], sem_o)

    def issue(i, p, part):
        h = p // nbg
        if isinstance(p, int):
            if p >= npair:
                return
            if part == 0:
                if p < nbg:
                    start_x(i, p)
                if p % nbg == 0:
                    start_w(i, h)
        elif part == 0:
            @pl.when(p % nbg == 0)
            def _():
                start_w(i, h)
        start_kv(i, p, part)

    def issue_pt(i, p, k):
        d, part = (k + SHIFT) // NPART, (k + SHIFT) % NPART
        issue((i + d) % 2, p + (i + d) // 2, part)

    deferred = []

    def flush():
        for k, (i, b) in enumerate(deferred):
            out_copy(i, b).start(priority=k % 2)
        deferred.clear()

    def item(i, p, final=None):
        static = isinstance(p, int)
        h, bg, slot = p // nbg, p % nbg, (2 * p + i) % nslot
        b0 = bg * nb
        r0 = row0(h)

        issue_pt(i, p, 0)
        if static:
            if p < nbg:
                wait_x(i, p)
            if bg == 0:
                wait_w(i, h)
        else:
            @pl.when(bg == 0)
            def _():
                wait_w(i, h)

        xc = jnp.concatenate(
            [x_v[i, kt, pl.ds(b0, nb)].reshape(nb * Sq, LANE) for kt in range(nkt)], axis=1)
        q = jnp.dot(xc, wq_v[i, h], preferred_element_type=jnp.float32)
        q = (q * c).astype(jnp.bfloat16)

        wait_kv(i, p)

        def qk(j):
            return jax.lax.dot_general(
                q[j * Sq:(j + 1) * Sq], kv_v[slot, 0, j], _NT,
                preferred_element_type=jnp.float32)

        outs = []
        s_next = qk(0)
        for j in range(nb):
            s = s_next
            if j + 1 < nb:
                s_next = qk(j + 1)
            m = jnp.max(s, axis=-1, keepdims=True)
            e = jnp.exp2(s - m)
            l = jnp.sum(e, axis=-1, keepdims=True)
            o = jnp.dot(e.astype(jnp.bfloat16), kv_v[slot, 1, j],
                        preferred_element_type=jnp.float32)
            o = (o * pl.reciprocal(l, approx=False)).astype(jnp.bfloat16)
            if j < NPART - 1:
                issue_pt(i, p, j + 1)
            if final is None:
                outs.append(o)
                continue
            b = b0 + j
            for jj in range(nkt):
                col = i * D + jj * LANE
                r = jnp.dot(o, wo_v[i, jj, pl.ds(r0, Dh), :],
                            preferred_element_type=jnp.float32)
                o_v[b, :, col:col + LANE] = (acc[b, :, col:col + LANE] + r).astype(o_v.dtype)
            deferred.append((i, b))
            if final == 'last' or (final == 'pen' and j >= FLUSH_J):
                flush()

        if final is None:
            oc = jnp.concatenate(outs, axis=0)
            for jj in range(nkt):
                col = i * D + jj * LANE
                r = jnp.dot(oc, wo_v[i, jj, pl.ds(r0, Dh), :],
                            preferred_element_type=jnp.float32)
                for j in range(nb):
                    acc[b0 + j, :, col:col + LANE] += r[j * Sq:(j + 1) * Sq]

    for g in range(SHIFT):
        t = g // NPART
        issue(t % 2, t // 2, g % NPART)
    acc[...] = jnp.zeros(acc.shape, acc.dtype)

    def step(p, carry):
        item(0, p)
        item(1, p)
        return carry

    n_tail = nbg + 1
    for p in range(nbg):
        step(p, 0)
    jax.lax.fori_loop(nbg, npair - n_tail, step, 0)
    for p in range(npair - n_tail, npair):
        for i in range(2):
            if p < npair - nbg:
                final = None
            elif p < npair - 1:
                final = 'defer'
            else:
                final = 'last' if i == 1 else 'pen'
            item(i, p, final)
    wait_all(o_v, sem_o)


@jax.jit
def pallas_concat_heads__mha_block_cached__gqa_block_cached__near_ridge_kernel(
    A_x: jax.Array,
    A_k_cache: jax.Array,
    A_v_cache: jax.Array,
    A_wq: jax.Array,
    A_wo: jax.Array,
    B_x: jax.Array,
    B_k_cache: jax.Array,
    B_v_cache: jax.Array,
    B_wq: jax.Array,
    B_wo: jax.Array,
):
    B, Sq, D = A_x.shape
    _, _, Sk, Dh = A_k_cache.shape
    H = A_wq.shape[1] // Dh
    assert B_x.shape == A_x.shape and B_wq.shape == A_wq.shape and B_wo.shape == A_wo.shape
    assert B_k_cache.shape[2:] == (Sk, Dh) and Dh == LANE
    assert B % NB == 0 and D % LANE == 0 and Sk % (CH * NPART) == 0 and NB == NPART
    reps = (H // A_k_cache.shape[1], H // B_k_cache.shape[1])
    nkt = D // LANE
    bf = jnp.bfloat16
    return pl.pallas_call(
        functools.partial(_kernel, B=B, Sq=Sq, D=D, H=H, Sk=Sk, Dh=Dh, reps=reps),
        in_specs=[pl.BlockSpec(memory_space=pl.ANY)] * 10,
        out_specs=pl.BlockSpec(memory_space=pl.ANY),
        out_shape=jax.ShapeDtypeStruct((B, Sq, 2 * D), bf),
        scratch_shapes=[
            pltpu.VMEM((2, nkt, B, Sq, LANE), bf),
            pltpu.VMEM((2, H, D, Dh), bf),
            pltpu.VMEM((2, nkt, H * Dh, LANE), bf),
            pltpu.VMEM((NSLOT, 2, NB, Sk, Dh), bf),
            pltpu.VMEM((B, Sq, 2 * D), jnp.float32),
            pltpu.VMEM((B, Sq, 2 * D), bf),
            pltpu.SemaphoreType.DMA((2 * NSLOT + 4 + 2 * (B // NB),)),
            pltpu.SemaphoreType.DMA(()),
        ],
        compiler_params=pltpu.CompilerParams(
            vmem_limit_bytes=100 * 1024 * 1024,
            disable_bounds_checks=True,
            disable_semaphore_checks=True),
    )(A_x, A_k_cache, A_v_cache, A_wq, A_wo,
      B_x, B_k_cache, B_v_cache, B_wq, B_wo)
```

```python
import functools
import math

import jax
import jax.numpy as jnp
import jax.experimental.pallas as pl
import jax.experimental.pallas.tpu as pltpu

_NT = (((1,), (1,)), ((), ()))
LANE = 128
NB = 4
CH = 32
NPART = 4
SHIFT = 8
NSLOT = 4
HG = 4
WQS = 4
WQR = 8
XR = 32
FLUSH_J = 1


def _kernel(xa, ka, va, wqa, woa, xb, kb, vb, wqb, wob,
            out,
            x_v, wq_v, wo_v, kv_v, acc, o_v,
            sems, sem_o,
            *, B, Sq, D, H, Sk, Dh, reps):
    nb, nslot = NB, NSLOT
    nbg = B // nb
    npair = H * nbg
    nkt = D // LANE
    cpp = Sk // CH // NPART
    gw = HG * Dh
    nwq = D // WQS // WQR
    wor = Dh // NPART
    c = (Dh ** -0.5) * math.log2(math.e)
    xs, wqs, wos = (xa, xb), (wqa, wqb), (woa, wob)
    ks, vs = (ka, kb), (va, vb)

    def sem_kv(slot, a):
        return sems.at[2 * slot + a]

    def sem_wq(i, par):
        return sems.at[2 * nslot + 2 * i + par]

    def sem_wo(i, par):
        return sems.at[2 * nslot + 4 + 2 * i + par]

    def sem_x(i, bg):
        return sems.at[2 * nslot + 8 + i * nbg + bg]

    def wait_all(view, sem):
        pltpu.make_async_copy(view, view, sem).wait()

    def mult(v, m):
        return v if isinstance(v, int) else pl.multiple_of(v, m)

    def start_x(i, bg):
        for j in range(nb):
            b = bg * nb + j
            for r in range(Sq // XR):
                pltpu.make_async_copy(
                    xs[i].at[b, pl.ds(r * XR, XR)], x_v.at[i, b, pl.ds(r * XR, XR)],
                    sem_x(i, bg)).start(priority=r % 2)

    def wait_x(i, bg):
        wait_all(x_v.at[i, pl.ds(bg * nb, nb)], sem_x(i, bg))

    def start_wq(i, g, k, prio):
        rr = mult(k * WQR, WQR)
        pltpu.make_async_copy(
            wqs[i].at[:, pl.ds(rr, WQR), pl.ds(mult(g * gw, gw), gw)],
            wq_v.at[i, g, :, pl.ds(rr, WQR)],
            sem_wq(i, g % 2)).start(priority=prio)

    def wait_wq(i, g):
        wait_all(wq_v.at[i, g], sem_wq(i, g % 2))

    def start_wo(i, h, part):
        pltpu.make_async_copy(
            wos[i].at[h, pl.ds(part * wor, wor)], wo_v.at[i, h, pl.ds(part * wor, wor)],
            sem_wo(i, h % 2)).start(priority=part % 2)

    def wait_wo(i, h):
        wait_all(wo_v.at[i, h], sem_wo(i, h % 2))

    def start_kv(i, p, part):
        h, bg, slot = p // nbg, p % nbg, (2 * p + i) % nslot
        hkv = h if reps[i] == 1 else h // reps[i]
        for ci in range(part * cpp, (part + 1) * cpp):
            for a, arr in enumerate((ks[i], vs[i])):
                pltpu.make_async_copy(
                    arr.at[pl.ds(bg * nb, nb), hkv, pl.ds(ci * CH, CH)],
                    kv_v.at[slot, a, :, pl.ds(ci * CH, CH)],
                    sem_kv(slot, a)).start(priority=a)

    def wait_kv(i, p):
        slot = (2 * p + i) % nslot
        for a in range(2):
            wait_all(kv_v.at[slot, a], sem_kv(slot, a))

    def out_copy(i, b):
        return pltpu.make_async_copy(
            o_v.at[b, :, pl.ds(i * D, D)], out.at[b, :, pl.ds(i * D, D)], sem_o)

    def issue(i, p, part):
        h, bg = p // nbg, p % nbg

        def wq_next():
            start_wq(i, h // HG + 1, (h % HG) * NPART + part, part % 2)

        if isinstance(p, int):
            if p >= npair:
                return
            if part == 0 and p < nbg:
                start_x(i, p)
            if part == 0 and p == 0:
                for k in range(nwq):
                    start_wq(i, 0, k, k % 2)
            if bg == 0:
                start_wo(i, h, part)
            elif bg == 1 and h < H - HG:
                wq_next()
        else:
            @pl.when(bg == 0)
            def _():
                start_wo(i, h, part)

            pl.when(jnp.logical_and(bg == 1, h < H - HG))(wq_next)
        start_kv(i, p, part)

    def issue_pt(i, p, k):
        d, part = (k + SHIFT) // NPART, (k + SHIFT) % NPART
        issue((i + d) % 2, p + (i + d) // 2, part)

    deferred = []

    def flush():
        for k, (i, b) in enumerate(deferred):
            out_copy(i, b).start(priority=k % 2)
        deferred.clear()

    def qproj(i, h, b0):
        xc = x_v[i, pl.ds(b0, nb)].reshape(nb * Sq, D)
        w = wq_v[i, h // HG, :, :, pl.ds(mult((h % HG) * Dh, Dh), Dh)].reshape(D, Dh)
        q = jnp.dot(xc, w, preferred_element_type=jnp.float32)
        return (q * c).astype(jnp.bfloat16)

    def item(i, p, final=None, pre=None, q_pre=None):
        static = isinstance(p, int)
        h, bg, slot = p // nbg, p % nbg, (2 * p + i) % nslot
        b0 = bg * nb

        def when(cond, fn):
            if static:
                if cond:
                    fn()
            else:
                pl.when(cond)(fn)

        issue_pt(i, p, 0)
        if static and p < nbg:
            wait_x(i, p)
        when(p % (HG * nbg) == 0, lambda: wait_wq(i, h // HG))

        q = qproj(i, h, b0) if q_pre is None else q_pre
        q_out = None if pre is None else qproj(*pre)

        wait_kv(i, p)
        when(bg == 0, lambda: wait_wo(i, h))

        def qk(j):
            return jax.lax.dot_general(
                q[j * Sq:(j + 1) * Sq], kv_v[slot, 0, j], _NT,
                preferred_element_type=jnp.float32)

        outs = []
        s_next = qk(0)
        for j in range(nb):
            s = s_next
            if j + 1 < nb:
                s_next = qk(j + 1)
            m = jnp.max(s, axis=-1, keepdims=True)
            e = jnp.exp2(s - m)
            l = jnp.sum(e, axis=-1, keepdims=True)
            o = jnp.dot(e.astype(jnp.bfloat16), kv_v[slot, 1, j],
                        preferred_element_type=jnp.float32)
            o = (o * pl.reciprocal(l, approx=False)).astype(jnp.bfloat16)
            if j < NPART - 1:
                issue_pt(i, p, j + 1)
            if final is None:
                outs.append(o)
                continue
            b = b0 + j
            for jj in range(nkt):
                col = i * D + jj * LANE
                r = jnp.dot(o, wo_v[i, h, :, jj * LANE:(jj + 1) * LANE],
                            preferred_element_type=jnp.float32)
                o_v[b, :, col:col + LANE] = (acc[b, :, col:col + LANE] + r).astype(o_v.dtype)
            deferred.append((i, b))
            if final == 'last' or (final == 'pen' and j >= FLUSH_J):
                flush()

        if final is None:
            oc = jnp.concatenate(outs, axis=0)
            for jj in range(nkt):
                col = i * D + jj * LANE
                r = jnp.dot(oc, wo_v[i, h, :, jj * LANE:(jj + 1) * LANE],
                            preferred_element_type=jnp.float32)
                for j in range(nb):
                    acc[b0 + j, :, col:col + LANE] += r[j * Sq:(j + 1) * Sq]
        return q_out

    for g in range(SHIFT):
        t = g // NPART
        issue(t % 2, t // 2, g % NPART)
    acc[...] = jnp.zeros(acc.shape, acc.dtype)

    def step(p, carry):
        item(0, p)
        item(1, p)
        return carry

    n_tail = nbg + 1
    for p in range(nbg):
        step(p, 0)
    jax.lax.fori_loop(nbg, npair - n_tail, step, 0)
    for p in range(npair - n_tail, npair - 1):
        for i in range(2):
            item(i, p, None if p < npair - nbg else 'defer')
    q_last = item(0, npair - 1, 'pen', pre=(1, H - 1, (nbg - 1) * nb))
    item(1, npair - 1, 'last', q_pre=q_last)
    wait_all(o_v, sem_o)


@jax.jit
def pallas_concat_heads__mha_block_cached__gqa_block_cached__near_ridge_kernel(
    A_x: jax.Array,
    A_k_cache: jax.Array,
    A_v_cache: jax.Array,
    A_wq: jax.Array,
    A_wo: jax.Array,
    B_x: jax.Array,
    B_k_cache: jax.Array,
    B_v_cache: jax.Array,
    B_wq: jax.Array,
    B_wo: jax.Array,
):
    B, Sq, D = A_x.shape
    _, _, Sk, Dh = A_k_cache.shape
    H = A_wq.shape[1] // Dh
    assert B_x.shape == A_x.shape and B_wq.shape == A_wq.shape and B_wo.shape == A_wo.shape
    assert B_k_cache.shape[2:] == (Sk, Dh) and Dh == LANE
    assert B == 2 * NB and D % LANE == 0 and Sk % (CH * NPART) == 0 and NB == NPART
    assert H % HG == 0 and D == WQS * WQR * HG * NPART
    reps = (H // A_k_cache.shape[1], H // B_k_cache.shape[1])
    bf = jnp.bfloat16
    wq_shape, wo_shape = (WQS, D // WQS, H * Dh), (H, Dh, D)
    return pl.pallas_call(
        functools.partial(_kernel, B=B, Sq=Sq, D=D, H=H, Sk=Sk, Dh=Dh, reps=reps),
        in_specs=[pl.BlockSpec(memory_space=pl.ANY)] * 10,
        out_specs=pl.BlockSpec(memory_space=pl.ANY),
        out_shape=jax.ShapeDtypeStruct((B, Sq, 2 * D), bf),
        scratch_shapes=[
            pltpu.VMEM((2, B, Sq, D), bf),
            pltpu.VMEM((2, H // HG, WQS, D // WQS, HG * Dh), bf),
            pltpu.VMEM((2, H, Dh, D), bf),
            pltpu.VMEM((NSLOT, 2, NB, Sk, Dh), bf),
            pltpu.VMEM((B, Sq, 2 * D), jnp.float32),
            pltpu.VMEM((B, Sq, 2 * D), bf),
            pltpu.SemaphoreType.DMA((2 * NSLOT + 8 + 2 * (B // NB),)),
            pltpu.SemaphoreType.DMA(()),
        ],
        compiler_params=pltpu.CompilerParams(
            vmem_limit_bytes=100 * 1024 * 1024,
            disable_bounds_checks=True,
            disable_semaphore_checks=True),
    )(A_x, A_k_cache, A_v_cache, A_wq.reshape(wq_shape), A_wo.reshape(wo_shape),
      B_x, B_k_cache, B_v_cache, B_wq.reshape(wq_shape), B_wo.reshape(wo_shape))
```
